```python
import os as _os
_os.environ.setdefault("JAX_PLATFORMS", "cpu")
import jax
import jax.numpy as jnp

def _softmax(x, axis=-1):
    return jax.nn.softmax(x, axis=axis)
def _gelu(x):
    return jax.nn.gelu(x, approximate=True)
def _silu(x):
    return jax.nn.silu(x)
def _sigmoid(x):
    return jax.nn.sigmoid(x)
def _layernorm(x, axis=-1, eps=1e-5):
    m = jnp.mean(x, axis=axis, keepdims=True)
    v = jnp.var(x, axis=axis, keepdims=True)
    return (x - m) / jnp.sqrt(v + eps)
def _scatter_add(tgt, idx, src, axis=0):
    return tgt.at[idx].add(src)
def _segment_sum(src, seg, n):
    return jax.ops.segment_sum(src, seg, n)
class _Rng:
    def __init__(self, key):
        self._k = key
    def _next(self):
        self._k, sub = jax.random.split(self._k)
        return sub
    def normal(self, shape):
        return jax.random.normal(self._next(), shape, dtype=jnp.bfloat16)
    def randint(self, lo, hi, shape):
        return jax.random.randint(self._next(), shape, lo, hi, dtype=jnp.int32)
    def uniform(self, shape, lo=0.0, hi=1.0):
        return jax.random.uniform(self._next(), shape, jnp.bfloat16, lo, hi)
    def permutation(self, n):
        return jax.random.permutation(self._next(), n)


kernel_name = 'standalone__mixer_token_mlp__sampling'

def setup_inputs():
    _rng = _Rng(jax.random.key(int.from_bytes(__import__("os").urandom(4), "little")))
    _w = (lambda a: (lambda t: t.astype(jnp.bfloat16) if jnp.issubdtype(t.dtype, jnp.floating) else t)(jnp.asarray(a)))
    B, S, D, F = 32, 16, 1024, 3584
    return {
        "x": _w((lambda *s: _rng.normal(s) * 0.05)(B, S, D)),
        "w1": _w((lambda *s: _rng.normal(s) * 0.05)(S, F) * (S ** -0.5)),
        "b1": _w((lambda *s: _rng.normal(s) * 0.05)(F) * 0.02),
        "w2": _w((lambda *s: _rng.normal(s) * 0.05)(F, S) * (F ** -0.5)),
        "b2": _w((lambda *s: _rng.normal(s) * 0.05)(S) * 0.02),
    }

def reference(x, w1, b1, w2, b2):
    B, S, D = x.shape
    h = _layernorm(x, axis=-1)
    u = jnp.einsum("bsd,sf->bdf", h, w1) + b1
    u = _gelu(u)
    y = jnp.einsum("bdf,fs->bds", u, w2) + b2
    return (lambda x, *d: x.transpose(*d))(y, 0, 2, 1)
```

```python
import jax, jax.numpy as jnp, numpy as np, functools, ml_dtypes
import jax.experimental.pallas as pl
import jax.experimental.pallas.tpu as pltpu

C1 = float(np.sqrt(2/np.pi)); C2 = C1*0.044715
SC = float(np.cbrt(C2)); KK = C1/SC
SC_HI = float(np.float32(SC).astype(ml_dtypes.bfloat16)); SC_LO = float(np.float32(SC-SC_HI).astype(ml_dtypes.bfloat16))
f32, bf16, u32 = jnp.float32, jnp.bfloat16, jnp.uint32
cat = jnp.concatenate

def make(LAG=3, flags=None, NB=32, N=15, HEAD=16, order='a', tree=2, hmode=1, W2W=3.0, LNW=0.4, LNO=3, LNN=3, TAIL=3,
         KM=8, UN=1, KS=2, HW=0.3, HN=2, lnm=1, ST=0, PAD=0, TW=1, AW=0.4, SG=(0,0,0,0), SGI=(), RP=2, ZS=0, RS=0):
    S, D, F, FC, DC, KP = 16, 1024, 3584, 128, 512, 32
    FO = 16*N; FM = F - FO
    NT = F // FC; NM = -(-FM // FC)
    nrows = [max(0, min(FC, FM - j*FC)) for j in range(NT)]
    work = [(d0, j) for d0 in range(0, D, DC) for j in range(NM)]
    NW = len(work); CARRY = LAG; NC = DC//128; NR = LAG + 1; NP = D//DC; NG = N + 1
    NS = 7 if ST else 2*KS; KL = 8 if ST else S//KS; JC = 2 if ST else 1
    jobs = [(g, c) for g in range(NG-1, -1, -1) for c in range(0, NC, JC)]
    cost = np.array(([16, 16 + 10*AW, 16, 17, 16 + 10*AW, 17 + 10*AW, 17 + 10*AW] if ST else [2*KL + (10*AW if q % KS == KS-1 else 0) for q in range(NS)]) * len(jobs), float)
    ccum = np.concatenate([[0], np.cumsum(cost)])
    O_H = (KL+1)*NG + PAD; O_D = O_H + NC; TROWS = 8*(((O_D + 2)//3 + 1) | 1)
    def slot(n): return slice(8*(n//3), 8*(n//3)+8), slice(128*(n % 3), 128*(n % 3)+128)
    def upk(x): return pltpu.bitcast(x, bf16)
    def put(view, val): view.bitcast(bf16)[...] = val.astype(bf16)
    nbg = len(jobs)*NS; LNI = NM + 4
    def mkplan(head, tail):
        plan = {}
        for p in range(NP):
            keys, wts = [], []
            for j in range(NM):
                i = p*NM + j
                for r in range(-2, nrows[j]//8):
                    for c in range(NC):
                        w = (W2W if r < 0 else 1.0) - (LNW if NW - LAG - LNO <= i < NW - LAG - LNO + LNN else 0) - (HW if head and CARRY <= i < CARRY + HN else 0)
                        if (i == CARRY - 1 and r >= 16 - tail) or (head and i == CARRY and r < 0): w = 0
                        keys.append((i, r, c)); wts.append(w)
            cum = np.cumsum(wts)/np.sum(wts); hd = ccum[head] if p == 0 else 0
            if p == 0:
                e = CARRY*18*NC; x0 = cum[e-1]*(ccum[-1] - hd); n0 = int(round(x0/ccum[NS]))*NS
                tgt = np.concatenate([cum[:e]/cum[e-1]*ccum[n0], ccum[n0] + hd + (cum[e:] - cum[e-1])/(1 - cum[e-1])*(ccum[-1] - ccum[n0] - hd)])
            else: tgt = cum*ccum[-1]
            for k, x in zip(keys, tgt): plan[k] = int(np.searchsorted(ccum, x - 1e-6))
        return plan
    plans = [mkplan(HEAD, TAIL)] + [mkplan(0, 0)]*(UN-1)
    def done_by(i): return plans[i // NW % UN][i % NW, nrows[work[i % NW][1]]//8 - 1, NC-1]
    def need(r0): return (NG - r0//16) * (NC//JC) * NS
    def kern(x_hbm, w1_ref, b1_ref, w2t_ref, b2_ref, o_hbm, x_ref, o_ref, w1p_ref, w2p_ref, hn_ref, lin_ref, xc_ref, sems, *rest):
        tabs = rest[:NS]; ring = rest[NS:NS+NR+CARRY]; gvs = rest[NS+NR+CARRY:-NP]; hps = rest[-NP:]
        def rg(i): return ring[NR + i % (NW*UN)] if i % (NW*UN) < CARRY else ring[i % NR]
        c0 = pltpu.make_async_copy(x_hbm.at[0:1], x_ref.at[0:1], sems.at[0]); c0.start()
        c1 = pltpu.make_async_copy(x_hbm.at[1:], x_ref.at[1:], sems.at[1]); c1.start()
        b1 = b1_ref[...].astype(f32).reshape(1, F)
        r = jax.lax.broadcasted_iota(jnp.int32, (8, F), 0)
        wa = cat([w1_ref[...].astype(f32), jnp.where(r < 2, jnp.broadcast_to(b1, (8, F)), 0.0)], axis=0)
        def tr(f0, f1): return cat([wa[:, f0:f1], jnp.zeros((128-S-8, f1-f0), f32)], axis=0).T
        f0 = FM//256*256
        wt = tr(f0, F)
        put(w1p_ref.at[0, :f0//2, :], tr(0, f0))
        if FM > f0: put(w1p_ref.at[0, f0//2:FM//2, :], wt[:FM-f0])
        wt = wt[FM-f0:]
        w2p_ref[0, :, :F] = w2t_ref.bitcast(u32)[...]
        b2 = jnp.broadcast_to(b2_ref[...].astype(f32).reshape(1, S), (S, S))
        eye = jax.lax.broadcasted_iota(jnp.int32, (S, S), 0) == jax.lax.broadcasted_iota(jnp.int32, (S, S), 1)
        b2c = jnp.sum(jnp.where(eye, b2, 0.0), axis=1, keepdims=True) * (2*SC)
        m = jax.lax.dot_general(w2t_ref[...], cat([wa, jnp.zeros((8, F), f32)], axis=0).astype(bf16), (((1,), (1,)), ((), ())), preferred_element_type=f32)
        if KM:
            sel = jax.lax.broadcasted_iota(jnp.int32, (KP, KM*128), 0) == jax.lax.broadcasted_iota(jnp.int32, (KP, KM*128), 1) // 128
            wm = jnp.dot(wt[:, :KP].astype(bf16), jnp.where(sel, 1.0, 0.0).astype(bf16), preferred_element_type=f32)
        cols = []
        for k in range(S+1):
            col = wm[:, 128*k:128*k+128] if k < KM else jnp.broadcast_to(wt[:, k:k+1], (FO, 128))
            mc = jnp.broadcast_to(m[:, k:k+1], (S, 128))
            if k == S: col = col * SC; mc = mc * SC + b2c
            cols.append([col[8*v:8*v+8] for v in range(2*N)] + [mc[:8], mc[8:]])
        for g in range(NG):
            if ST:
                for k in range(8):
                    a11, a12, a21, a22 = cols[k][2*g], cols[k+8][2*g], cols[k][2*g+1], cols[k+8][2*g+1]
                    s1 = a21 + a22; s2 = s1 - a11
                    for q, val in enumerate([a11, a12, s2, a11 - a21, a22, s1, a12 - s2]): tabs[q][(0,) + slot(g*(KL+1) + k)] = val
                tabs[0][(0,) + slot(g*(KL+1) + KL)] = cols[S][2*g]
                tabs[3][(0,) + slot(g*(KL+1) + KL)] = cols[S][2*g+1] - cols[S][2*g]
            else:
                for q in range(NS):
                    for k in range(KL): tabs[q][(0,) + slot(g*(KL+1) + k)] = cols[q % KS*KL + k][2*g + q//KS]
                    if q % KS == 0: tabs[q][(0,) + slot(g*(KL+1) + KL)] = cols[S][2*g + q//KS]
        r = jax.lax.broadcasted_iota(jnp.int32, (KP-S, DC), 0)
        for hp in hps: put(hp.at[0, S//2:KP//2, :DC], jnp.where(r == 0, SC_HI, jnp.where(r == 1, SC_LO, 0.0)))

        def ln(b, z0=0):
            x = upk(x_ref.bitcast(u32)[b]).astype(f32)
            m = jnp.mean(x, axis=-1, keepdims=True)
            if lnm: x = upk(x_ref.bitcast(u32)[b + z0]).astype(f32)
            xc = x - m
            v = jnp.mean(xc*xc, axis=-1, keepdims=True)
            if lnm: xc_ref[z0] = xc; xc = xc_ref[0]
            put(hn_ref.at[z0], xc * (SC*jax.lax.rsqrt(v + 1e-5)))
        def put_h(d0, z0=0): hps[d0//DC][z0, :S//2, :DC] = hn_ref[0, :, d0:d0+DC]
        def act(u): return u * jnp.tanh(u * (u*u + KK))
        def bg(st, d0, z0, z1, key, s):
            n, q = divmod(st, NS)
            g, c = jobs[n]; t = tabs[q]
            if key is not None: t[(z0,) + slot(O_D)] = key
            if g == NG-1:
                hc = upk(hn_ref[0, :, d0+128*c:d0+128*(c+JC)]).astype(f32)
                if ST:
                    b11, b12, b21, b22 = hc[:8, :128], hc[:8, 128:], hc[8:, :128], hc[8:, 128:]
                    hq = [b11, b21, b22 - (b12 - b11), b22 - b12, b21 - (b22 - (b12 - b11)), b12 - b11, b22][q]
                else: hq = hc[q % KS*KL//8*8:][:8]
                t[(z1,) + slot(O_H + c)] = hq
            def mac(*init):
                rs, cs = slot(O_H + c); r0 = rs.start + (0 if ST else q % KS*KL % 8)
                parts = list(init) + [None]*(tree - len(init))
                for k in range(KL):
                    p = t[(0,) + slot(g*(KL+1) + k)] * t[0, r0+k:r0+k+1, cs]
                    e = (k + 1) % len(parts)
                    parts[e] = p if parts[e] is None else parts[e] + p
                return functools.reduce(lambda a, b: a + b, parts)
            bias = lambda: t[(0,) + slot(g*(KL+1) + KL)]
            def fin(a): return a if g == NG-1 else act(a)
            def out(cc, a0, a1):
                cs = slice(128*cc, 128*cc+128); f = FM + 16*g
                if g == NG-1: lin_ref[z0, :, cs] = cat([a0, a1], axis=0)
                else: put(gvs[f//FC - FM//FC].at[z0, f % FC//2:f % FC//2 + 8, cs], cat([a0, a1], axis=0))
            if ST:
                if q == 0: a = s['p1'] = mac(bias())
                if q == 1: a = s['c11'] = fin(mac(s['p1']))
                if q == 2: a = s['u2'] = mac(s['p1'])
                if q == 3: a = s['u3'] = mac(s['u2'], bias())
                if q == 4: a = fin(mac(s['u3'])); out(c, s['c11'], a)
                if q == 5: p5 = mac(); s['u4'] = s['u2'] + p5; a = s['c22'] = fin(s['u3'] + p5)
                if q == 6: a = fin(mac(s['u4'])); out(c+1, a, s['c22'])
            else:
                a = s['a'] = mac(bias() if q % KS == 0 else s['a'])
                if q == KS-1: a = s['lo'] = fin(a)
                if q == NS-1: a = fin(a); out(c, s['lo'], a)
            if key is None: t[(z1,) + slot(O_D + 1)] = a
        def mm1(i, s, p, z0=0, z1=0, zh=0):
            d0, j = work[i % NW]
            if j == 0 and i: w1p_ref[z0, F//2:, :] = jnp.zeros((8, 128), u32)
            lhs = upk(w1p_ref[0, j*FC//2:(j*FC+nrows[j])//2, :])[:, :KP]
            rhs = hps[d0//DC][0, :KP//2, :DC]
            if any(SG) and (i == CARRY or i in SGI):
                ps = []
                for c in range(NC):
                    z = 0
                    for _ in range(SG[c]): z = (z0 if isinstance(z, int) else z) >> z1
                    ps.append(hps[d0//DC][z, :KP//2, 128*c:128*c+128])
                rhs = cat(ps, axis=1)
            u = jnp.dot(lhs, upk(rhs), preferred_element_type=f32)
            n = done_by(i-1) if j else 0
            for r in range(-2, nrows[j]//8):
                for c in range(NC):
                    while n < plans[i // NW % UN][i % NW, r, c]:
                        src = u[8*r:8*r+8] if r >= 0 else None if p is None else p[8*r+16:8*r+24]
                        bg(n, d0, z0, z1, None if src is None else src[:, 128*c:128*c+128], s); n += 1
            put(rg(i).at[0 if RS else z0, :nrows[j]//2, :], act(u))
            if hmode and i % (NW*UN) != CARRY-1 and j != NM-1: hps[d0//DC][z0, KP//2:, :128] = rhs[:8, :128]
        def mm2(j, g, zh):
            return jnp.dot(upk(w2p_ref[0, :, j*FC:(j+1)*FC]), upk(g), preferred_element_type=f32)
        c0.wait()
        ln(0); put_h(0)
        s = {}
        for i in range(CARRY): mm1(i, s, None)
        c1.wait()

        def body(t, _):
            z0 = (t >> 10) << ZS; z1 = (t >> 11) << ZS
            zh = lambda i: (t >> (12 + i // NM)) << ZS
            s = {}; nxt = [CARRY]; p = None
            def issue(upto):
                while nxt[0] <= min(upto, NW*UN+CARRY-1):
                    i = nxt[0]; nxt[0] += 1
                    if i % NW == CARRY:
                        for d0 in range(DC, D, DC): put_h(d0, z0)
                    mm1(i, s, p, z0, z1, zh(i))
                    if i % NW == LNI: ln(jnp.minimum(t*UN + i//NW + 1, NB-1), z0); put_h(0, z0)
            acc = None
            for i, (d0, j) in enumerate(work*UN):
                if j == 0 and i: w2p_ref[z0, :, F:] = jnp.zeros((8, 128), u32)
                if j == 0: todo = list(range(NT-1, NM-1, -1)); lin = True
                last = (i == NW*UN-1 and order == 'b')
                extra = []
                if j == NM-1 and nrows[j] < FC: extra = [gvs[0][0, nrows[j]//2:, :]]
                issue(i+LAG-(1 if last else 0))
                p = mm2(j, cat([rg(i)[z0 if RS else 0, :nrows[j]//2, :]] + extra, axis=0), zh(i))
                acc = p if j == 0 else acc + p
                if lin and done_by(i) >= need(FO): acc = acc + lin_ref[0]; lin = False
                while todo and done_by(i) >= need(todo[0]*FC - FM):
                    jj = todo.pop(0); acc = acc + mm2(jj, gvs[jj - FM//FC][0], zh(i))
                if j == NM-1:
                    assert not todo and not lin
                    o_ref[t*UN + i//NW, :, d0:d0+DC] = (acc * (0.5/SC)).astype(o_ref.dtype)
            pltpu.make_async_copy(o_ref.at[pl.ds(t*UN, UN)], o_hbm.at[pl.ds(t*UN, UN)], sems.at[2]).start()
            issue(NW*UN+CARRY)
        jax.lax.fori_loop(0, NB//UN, body, None)
        pltpu.make_async_copy(o_ref.at[0:NB], o_hbm.at[0:NB], sems.at[2]).wait()
    @jax.jit
    def pallas_standalone__mixer_token_mlp__sampling_kernel(x, w1, b1, w2, b2):
        vm = pl.BlockSpec(memory_space=pltpu.VMEM)
        return pl.pallas_call(kern,
            in_specs=[pl.BlockSpec(memory_space=pl.ANY), vm, vm, vm, vm],
            out_specs=pl.BlockSpec(memory_space=pl.ANY),
            out_shape=jax.ShapeDtypeStruct(x.shape, x.dtype),
            scratch_shapes=[pltpu.VMEM(x.shape, x.dtype), pltpu.VMEM(x.shape, x.dtype), pltpu.VMEM((2, F//2 + 8, 128), u32), pltpu.VMEM((2, S//2, F + 128), u32),
                            pltpu.VMEM((2, S//2, D), u32), pltpu.VMEM((2, S, DC), f32), pltpu.VMEM((2, S, D), f32), pltpu.SemaphoreType.DMA((3,))]
                           + [pltpu.VMEM((2, TROWS, 384), f32)]*NS + [pltpu.VMEM((RP, FC//2, DC), u32)]*(NR+CARRY+NT - FM//FC) + [pltpu.VMEM((2, KP//2 + 8, DC + 128), u32)]*NP,
            compiler_params=pltpu.CompilerParams(vmem_limit_bytes=64*2**20, flags=flags),
        )(x, w1, b1, w2.T, b2)
    return pallas_standalone__mixer_token_mlp__sampling_kernel

pallas_standalone__mixer_token_mlp__sampling_kernel = make(N=15, W2W=1, hmode=0)
```

```python
import functools

import jax
import jax.experimental.pallas as pl
import jax.experimental.pallas.tpu as pltpu
import jax.numpy as jnp
import numpy as np

f32, bf16, u32 = jnp.float32, jnp.bfloat16, jnp.uint32
cat = jnp.concatenate

_C = float(np.sqrt(2 / np.pi))
_SCALE = float(np.cbrt(_C * 0.044715))
_SHIFT = _C / _SCALE
_SCALE_HI = float(np.float32(_SCALE).astype(bf16))
_SCALE_LO = float(np.float32(_SCALE - _SCALE_HI).astype(bf16))

TILE = 128
COLS = 512
KPAD = 32
STEPS = 7

_TUNING = dict(
    groups=18,
    unroll=2,
    lag=3,
    ahead=6,
    head=16,
    skip=4,
    loose=3,
    tail=6,
    w_out=0.75,
    w_extra=0.5,
    n_extra=2,
    w_norm=0.19,
    w_tilt=0.01,
    norm_at=0,
    norm_by=6,
    next_at=16,
    mixed_at=9,
    chains=2,
    mxu_pairs=5,
)


def _packed(words):
    return pltpu.bitcast(words, bf16)


def _pack_into(view, val):
    view.bitcast(bf16)[...] = val.astype(bf16)


def _act(v):
    return v * jnp.tanh(v * (v * v + _SHIFT))


def _slot(n, plane=0):
    r, c = 8 * (n // 3), 128 * (n % 3)
    return plane, slice(r, r + 8), slice(c, c + 128)


def _build(B, S, D, F, *, groups, unroll, lag, ahead, head, skip, loose, tail, w_out, w_extra, n_extra,
           w_norm, w_tilt, norm_at, norm_by, next_at, mixed_at, chains, mxu_pairs):
    assert S == 16 and D == 2 * COLS and F % (2 * TILE) == 0
    assert B % unroll == 0 and 2 * unroll < B < 1024
    lanes = COLS // 128
    f_mxu = F - 16 * groups
    n_tiles, mixed = F // TILE, f_mxu // TILE
    assert f_mxu % TILE
    order = [*range(mixed_at), mixed, *range(mixed_at, mixed)]
    per_pass = len(order)
    per_batch = 2 * per_pass
    assert lag + norm_at <= norm_by < per_pass and 0 < next_at <= per_pass and lag <= mixed_at
    n_items = unroll * per_batch

    def item(i):
        j = order[i % per_pass]
        return i // per_pass % 2 * COLS, j, min(TILE, f_mxu - j * TILE)

    jobs = [(g, c) for g in [groups, *range(groups)] for c in range(0, lanes, 2)]
    pass_steps = STEPS * len(jobs)
    first = STEPS * ahead
    cost = [16 + e + (a if g < groups else 0) for g, _ in jobs
            for e, a in zip([0, 0, 0, 1, 0, 1, 0], [0, 5, 0, 0, 6, 5, 6])]
    spent = np.cumsum([0] + cost * (2 * unroll + 1))

    def needed(i, j):
        done = 1 + ((j + 1) * TILE - f_mxu) // 16
        return i // per_pass * pass_steps + STEPS * lanes // 2 * done

    def spread(extra):
        keys, weights = [], []
        for i in range(lag, n_items + lag):
            for r in range(-2, item(i)[2] // 8):
                w = (w_out if r < 0 else 1.0) + (w_extra if i in extra and r < n_extra else 0)
                w -= w_norm if norm_by - 1 <= i % per_batch <= norm_by + 1 else 0
                w -= w_tilt * i / n_items
                if (i == lag and r < 0) or (i == n_items + lag - 1 and r >= 16 - tail):
                    w = 0
                keys += [(i, r, c) for c in range(lanes)]
                weights += [w] * lanes
        lo, hi = spent[first + head + loose], spent[first + 2 * unroll * pass_steps]
        target = lo + np.cumsum(weights) / np.sum(weights) * (hi - lo) - 1e-6
        return dict(zip(keys, np.searchsorted(spent, target).tolist()))

    def released(i):
        return plan[i, item(i)[2] // 8 - 1, lanes - 1] if i >= lag else first

    def consumers():
        return {next(i for i in range(p, p + per_pass) if released(i - 1) >= needed(i, j)): j
                for p in range(0, n_items, per_pass) for j in range(mixed + 1, n_tiles)}

    plan = spread(())
    plan = spread([i + lag + 1 for i in consumers()])
    vpu_tile_at = consumers()
    assert len(vpu_tile_at) == 2 * unroll * (n_tiles - mixed - 1)
    assert first <= needed(0, mixed + 1)

    h_slot = 9 * (groups + 1)
    mark = h_slot + D // 128
    lin_row = TILE

    def kernel(x_hbm, x0_ref, w1_ref, b1_ref, w2t_ref, b2_ref, o_hbm,
               x_ref, o_ref, w1p_ref, w2p_ref, normed, tables, ring, vpu_out, rhs, sems):
        x_next = pltpu.make_async_copy(x_hbm.at[unroll:2 * unroll], x_ref.at[unroll:2 * unroll], sems.at[0])
        x_rest = pltpu.make_async_copy(x_hbm.at[2 * unroll:], x_ref.at[2 * unroll:], sems.at[1])
        o_most = pltpu.make_async_copy(o_ref.at[:B - unroll], o_hbm.at[:B - unroll], sems.at[2])
        o_last = pltpu.make_async_copy(o_ref.at[B - unroll:], o_hbm.at[B - unroll:], sems.at[3])
        x_next.start()
        x_rest.start()


        def layernorm(x, h_ref, z0=0):
            x = x.astype(f32)
            xc = x - jnp.mean(x, axis=-1, keepdims=True)
            var = jnp.mean(xc * xc, axis=-1, keepdims=True)
            h = xc * (_SCALE * jax.lax.rsqrt(var + 1e-5))
            _pack_into(h_ref.at[z0, :, :D], h)
            return h

        def to_mxu(p, z0=0):
            rhs[p][z0, :S // 2, :] = normed[p // 2][0, :, p % 2 * COLS:(p % 2 + 1) * COLS]

        def to_vpu(p, z1=0):
            for d in range(p % 2 * COLS, (p % 2 + 1) * COLS, 256):
                h = _packed(normed[p // 2][0, :, d:d + 256]).astype(f32)
                b11, b12, b21, b22 = h[:8, :128], h[:8, 128:], h[8:, :128], h[8:, 128:]
                t1 = b12 - b11
                t2 = b22 - t1
                for table, val in zip(tables, [b11, b21, t2, b22 - b12, b21 - t2, t1, b22]):
                    table[_slot(h_slot + d // 128, z1)] = val

        def vpu_rows(j):
            return (vpu_out[0], (j - mixed) * TILE // 2) if j <= mixed + 1 else (vpu_out[j - mixed - 1], 0)

        def vpu_step(n, live, after=None, z0=0):
            g, c = jobs[n % pass_steps // STEPS]
            q = n % STEPS
            table = tables[q]
            if after is not None:
                table[_slot(mark, z0)] = after
            _, rows, cols = _slot(h_slot + n // pass_steps % 2 * lanes + c)
            parts = [live[k] for k in [[], ["p1"], ["p1"], ["u2"], ["u3"], [], ["u4"]][q]]
            parts += [table[_slot(9 * g + 8)]] if q in (0, 3) else []
            parts += [None] * (chains - len(parts))
            for k in range(8):
                p = table[_slot(9 * g + k)] * table[0, rows.start + k:rows.start + k + 1, cols]
                e = (k + 1) % len(parts)
                parts[e] = p if parts[e] is None else parts[e] + p
            a = functools.reduce(jnp.add, parts)
            if q == 5:
                live["u4"] = live["u2"] + a
                a = live["u3"] + a
            name = ["p1", "c11", "u2", "u3", "c21", "c22", "c12"][q]
            live[name] = _act(a) if name[0] == "c" and g < groups else a
            if q in (4, 6):
                col = 1 if q == 4 else 2
                out = cat([live[f"c1{col}"], live[f"c2{col}"]], axis=0)
                cols = slice(128 * (c + col - 1), 128 * (c + col))
                if g == groups:
                    vpu_out[0][z0, lin_row:lin_row + S, cols] = pltpu.bitcast(out, u32)
                else:
                    j, r = divmod(f_mxu + 16 * g, TILE)
                    ref, r0 = vpu_rows(j)
                    _pack_into(ref.at[z0, r0 + r // 2:r0 + r // 2 + 8, cols], out)
            return a

        def staged(i):
            i %= n_items
            return ring[i] if i < lag else ring[lag + i % (lag + 1)]

        def layer1(i, live, prev=None, z0=0, z1=0):
            _, j, rows = item(i)
            n = released(i - 1)
            if i % per_pass == 0 and i:
                w1p_ref[z0, TILE // 2:, :128] = jnp.zeros((8, 128), u32)
            lhs = []
            for r in range(rows // 16):
                while i == lag and n < first + head * max(0, r + 1 - skip) // (8 - skip):
                    c = 128 * (n % 8)
                    w1p_ref[z0, TILE // 2:, c:c + 128] = pltpu.bitcast(vpu_step(n, live, z0=z0), u32)
                    n += 1
                lhs.append(w1p_ref[0, 8 * r:8 * r + 8, j * TILE:(j + 1) * TILE])
            for _ in range(loose if i == lag else 0):
                tables[n % STEPS][_slot(mark + 1, z1)] = vpu_step(n, live, z0=z0)
                n += 1
            v = jnp.dot(_packed(cat(lhs, axis=0))[:, :KPAD], _packed(rhs[i // per_pass % len(rhs)][0]),
                        preferred_element_type=f32)
            for r in range(-2, rows // 8):
                for c in range(lanes):
                    while n < plan.get((i, r, c), 0):
                        src = v[8 * r:8 * r + 8] if r >= 0 else prev[8 * r + 16:8 * r + 24]
                        vpu_step(n, live, src[:, 128 * c:128 * c + 128], z0)
                        n += 1
            _pack_into(staged(i).at[z0, :rows // 2, :], _act(v))
            if j == mixed:
                assert needed(i, j) <= n <= (i // per_pass + 1) * pass_steps
                live["rest"] = vpu_out[0][0, rows // 2:TILE // 2, :COLS]
                live["lin"] = pltpu.bitcast(vpu_out[0][0, lin_row:lin_row + S, :COLS], f32)
            if i in vpu_tile_at:
                j = vpu_tile_at[i]
                assert n <= (needed(i + per_pass, j - 1) if j > mixed + 1 else (i // per_pass + 1) * pass_steps)
                ref, r0 = vpu_rows(j)
                live["tile"] = ref[0, r0:r0 + TILE // 2, :COLS]

        def layer2(j, words):
            return jnp.dot(_packed(w2p_ref[0, :, j * TILE:(j + 1) * TILE]), _packed(words),
                           preferred_element_type=f32)

        for b, h_ref in enumerate(normed):
            layernorm(x0_ref[b], h_ref)
        to_mxu(0)
        to_vpu(0)
        row = jax.lax.broadcasted_iota(jnp.int32, (8, F), 0)
        b1 = jnp.broadcast_to(b1_ref[...].astype(f32).reshape(1, F), (8, F))
        w1 = cat([w1_ref[...].astype(f32), jnp.where(row < 2, b1, 0.0)], axis=0)
        row = jax.lax.broadcasted_iota(jnp.int32, (KPAD - S, COLS), 0)
        for ref in rhs:
            _pack_into(ref.at[0, S // 2:, :], jnp.where(row == 0, _SCALE_HI, jnp.where(row == 1, _SCALE_LO, 0.0)))

        def transpose(f0, f1):
            wt = cat([w1[:, f0:f1], jnp.zeros((128 - S - 8, f1 - f0), f32)], axis=0).T
            for f in range(f0, min(f1, f_mxu), TILE):
                _pack_into(w1p_ref.at[0, :TILE // 2, f:f + TILE], wt[f - f0:f - f0 + TILE])
            return wt

        f0 = f_mxu // 256 * 256
        w_vpu = transpose(f0, F)[f_mxu - f0:]
        transpose(0, f0)
        w2t = w2t_ref[...]
        w2p_ref[0, :, :F] = pltpu.bitcast(w2t, u32)
        w21 = jax.lax.dot_general(w2t, cat([w1, jnp.zeros((8, F), f32)], axis=0).astype(bf16),
                                  (((1,), (1,)), ((), ())), preferred_element_type=f32)
        eye = jax.lax.broadcasted_iota(jnp.int32, (S, S), 0) == jax.lax.broadcasted_iota(jnp.int32, (S, S), 1)
        b2 = jnp.broadcast_to(b2_ref[...].astype(f32).reshape(1, S), (S, S))
        b2 = jnp.sum(jnp.where(eye, b2, 0.0), axis=1, keepdims=True)
        shape = (KPAD, 256 * mxu_pairs)
        t = jax.lax.broadcasted_iota(jnp.int32, shape, 1) >> 7
        pick = jax.lax.broadcasted_iota(jnp.int32, shape, 0) == (t >> 1) + 8 * (t & 1)
        picked = jnp.dot(w_vpu[:, :KPAD].astype(bf16), jnp.where(pick, 1.0, 0.0).astype(bf16),
                         preferred_element_type=f32)

        def column(k, g):
            if g < groups and k < S and k % 8 < mxu_pairs:
                return picked[16 * g:16 * g + 16, 256 * (k % 8) + 128 * (k // 8):][:, :128]
            w = w_vpu[16 * g:16 * g + 16] if g < groups else w21
            return jnp.broadcast_to(w[:, k:k + 1], (16, 128))

        for g in range(groups + 1):
            bias = column(S, g) * _SCALE
            if g == groups:
                bias = bias + b2 * (2 * _SCALE)
            tables[0][_slot(9 * g + 8)] = bias[:8]
            tables[3][_slot(9 * g + 8)] = bias[8:] - bias[:8]
        for g in range(groups + 1):
            for k in range(8):
                lo, hi = column(k, g), column(k + 8, g)
                a11, a21, a12, a22 = lo[:8], lo[8:], hi[:8], hi[8:]
                s1 = a21 + a22
                s2 = s1 - a11
                for table, val in zip(tables, [a11, a12, s2, a11 - a21, a22, s1, a12 - s2]):
                    table[_slot(9 * g + k)] = val
        vpu_out[0][0, :S, COLS:] = pltpu.bitcast(jnp.full((S, 128), 0.5 / _SCALE, f32), u32)

        live = {}
        for n in range(first):
            vpu_step(n, live)
        for i in range(lag):
            layer1(i, live)
        x_next.wait()

        def body(t, carry):
            z0, z1 = t >> 10, t >> 11
            live, part, scale = {}, None, 0.5 / _SCALE
            for p in range(1, 2 * unroll):
                to_mxu(p, z0)
            for i in range(n_items):
                batch, phase = divmod(i + lag, per_batch)
                if phase == lag + norm_at:
                    assert released(i + lag - 1) // pass_steps == 2 * batch
                    to_vpu(2 * batch + 1, z1)
                    h = layernorm(x_ref[jnp.minimum((t + 1) * unroll + batch, B - 1)], normed[batch], z0)
                if phase == norm_by:
                    for e in range(2):
                        tables[0][_slot(mark + e, z1)] = h[8 * e:8 * e + 8, -128:]
                if phase == per_batch - next_at:
                    assert released(i + lag - 1) // pass_steps == 2 * batch + 1
                    if batch == unroll - 1:
                        normed[0][z1, :, D:] = pltpu.bitcast(part[:8, :128], u32)
                        to_mxu(0, z0)
                    to_vpu((2 * batch + 2) % (2 * unroll), z1)
                if i == n_items - 1:
                    scale = cat([pltpu.bitcast(vpu_out[0][0, :S, COLS:], f32)] * lanes, axis=1)
                layer1(i + lag, live, part, z0, z1)

                d0, j, rows = item(i)
                if i % per_pass == 0 and i:
                    w2p_ref[z0, :, F:] = jnp.zeros((8, 128), u32)
                words = staged(i)[0, :rows // 2, :]
                part = layer2(j, cat([words, live.pop("rest")], axis=0) if j == mixed else words)
                acc = part if i % per_pass == 0 else acc + part
                if j == mixed:
                    acc = acc + live.pop("lin")
                if i in vpu_tile_at:
                    acc = acc + layer2(vpu_tile_at[i], live.pop("tile"))
                if i % per_pass == per_pass - 1:
                    o_ref[t * unroll + i // per_batch, :, d0:d0 + COLS] = (acc * scale).astype(o_ref.dtype)
            pl.when(t == 0)(x_rest.wait)
            pl.when(t == B // unroll - 2)(o_most.start)
            return carry

        jax.lax.fori_loop(0, B // unroll, body, None)
        o_last.start()
        o_most.wait()
        o_last.wait()

    def words(*shape):
        return pltpu.VMEM((2, *shape), u32)

    scratch = [
        pltpu.VMEM((B, S, D), bf16),
        pltpu.VMEM((B, S, D), bf16),
        words(TILE // 2 + 8, F + 128),
        words(S // 2, F + 128),
        [words(S // 2, D + 128)] * unroll,
        [pltpu.VMEM((2, 8 * ((mark + 1) // 3 + 1 | 1), 384), f32)] * STEPS,
        [words(TILE // 2, COLS)] * (2 * lag + 1),
        [words(lin_row + S + 8, COLS + 128)] + [words(TILE // 2, COLS)] * (n_tiles - mixed - 2),
        [words(KPAD // 2, COLS)] * (2 * unroll),
        pltpu.SemaphoreType.DMA((4,)),
    ]
    return kernel, scratch


@jax.jit
def pallas_standalone__mixer_token_mlp__sampling_kernel(
    x: jax.Array,
    w1: jax.Array,
    b1: jax.Array,
    w2: jax.Array,
    b2: jax.Array,
):
    B, S, D = x.shape
    kernel, scratch = _build(B, S, D, w1.shape[1], **_TUNING)
    whole = pl.BlockSpec(memory_space=pltpu.VMEM)
    return pl.pallas_call(
        kernel,
        grid=(1,),
        in_specs=[
            pl.BlockSpec(memory_space=pl.ANY),
            pl.BlockSpec((_TUNING["unroll"], S, D), lambda i: (0, 0, 0)),
            whole,
            whole,
            whole,
            whole,
        ],
        out_specs=pl.BlockSpec(memory_space=pl.ANY),
        out_shape=jax.ShapeDtypeStruct(x.shape, x.dtype),
        scratch_shapes=scratch,
        compiler_params=pltpu.CompilerParams(vmem_limit_bytes=48 * 2**20),
    )(x, x, w1, b1, w2.T, b2)
```
